```python
import os as _os
_os.environ.setdefault("JAX_PLATFORMS", "cpu")
import jax
import jax.numpy as jnp

def _softmax(x, axis=-1):
    return jax.nn.softmax(x, axis=axis)
def _gelu(x):
    return jax.nn.gelu(x, approximate=True)
def _silu(x):
    return jax.nn.silu(x)
def _sigmoid(x):
    return jax.nn.sigmoid(x)
def _layernorm(x, axis=-1, eps=1e-5):
    m = jnp.mean(x, axis=axis, keepdims=True)
    v = jnp.var(x, axis=axis, keepdims=True)
    return (x - m) / jnp.sqrt(v + eps)
def _scatter_add(tgt, idx, src, axis=0):
    return tgt.at[idx].add(src)
def _segment_sum(src, seg, n):
    return jax.ops.segment_sum(src, seg, n)
class _Rng:
    def __init__(self, key):
        self._k = key
    def _next(self):
        self._k, sub = jax.random.split(self._k)
        return sub
    def normal(self, shape):
        return jax.random.normal(self._next(), shape, dtype=jnp.bfloat16)
    def randint(self, lo, hi, shape):
        return jax.random.randint(self._next(), shape, lo, hi, dtype=jnp.int32)
    def uniform(self, shape, lo=0.0, hi=1.0):
        return jax.random.uniform(self._next(), shape, jnp.bfloat16, lo, hi)
    def permutation(self, n):
        return jax.random.permutation(self._next(), n)


kernel_name = 'standalone__linear_kernel_rfa__decode'

def setup_inputs():
    _rng = _Rng(jax.random.key(int.from_bytes(__import__("os").urandom(4), "little")))
    _w = (lambda a: (lambda t: t.astype(jnp.bfloat16) if jnp.issubdtype(t.dtype, jnp.floating) else t)(jnp.asarray(a)))
    B, H, Sq, Sk, D, M = 2, 16, 1, 16384, 256, 16
    return {
        "q": _w((lambda *s: _rng.normal(s) * 0.4)(B, H, Sq, D)),
        "k": _w((lambda *s: _rng.normal(s) * 1.6)(B, H, Sk, D)),
        "v": _w((lambda *s: _rng.normal(s) * 1.6)(B, H, Sk, D)),
        "omega": _w((lambda *s: _rng.normal(s) * 1.6)(M, D)),
    }

def reference(q, k, v, omega):
    d = q.shape[-1]
    m = omega.shape[0]
    scale = float(d) ** -0.25
    qs = q * scale
    ks = k * scale
    q_proj = jnp.einsum("bhsd,md->bhsm", qs, omega)
    k_proj = jnp.einsum("bhsd,md->bhsm", ks, omega)
    q_sq = 0.5 * jnp.einsum("bhsd,bhsd->bhs", qs, qs)[..., None]
    k_sq = 0.5 * jnp.einsum("bhsd,bhsd->bhs", ks, ks)[..., None]
    inv_sqrt_m = float(m) ** -0.5
    phi_q = jnp.exp(q_proj - q_sq) * inv_sqrt_m + 1e-6
    phi_k = jnp.exp(k_proj - k_sq) * inv_sqrt_m + 1e-6
    kv = jnp.einsum("bhsm,bhsd->bhmd", phi_k, v)
    z  = jnp.einsum("bhsm->bhm", phi_k)
    num = jnp.einsum("bhqm,bhmd->bhqd", phi_q, kv)
    den = jnp.einsum("bhqm,bhm->bhq", phi_q, z)[..., None] + 1e-6
    return num / den
```

```python
import functools

import jax
import jax.numpy as jnp
import jax.experimental.pallas as pl
import jax.experimental.pallas.tpu as pltpu

_NT = (((1,), (1,)), ((), ()))
_NN = (((1,), (0,)), ((), ()))

_R = 1024
_SUB = 64
_NSLOT = 4


def _rfa_kernel(q_ref, om_ref, k_hbm, v_hbm, o_ref, kbuf, vbuf, sems, acc, zacc, *, Sk):
    D = k_hbm.shape[-1]
    M = om_ref.shape[0]
    R, r, nslot = _R, _SUB, _NSLOT
    nsub = R // r
    bph = Sk // R
    n = k_hbm.shape[0] // R
    scale = float(D) ** -0.25
    ism = float(M) ** -0.5

    def start(i, slot):
        base = i * R
        for j in range(nsub):
            pltpu.make_async_copy(
                k_hbm.at[pl.ds(base + j * r, r)], kbuf.at[slot, pl.ds(j * r, r)],
                sems.at[0, slot]).start(priority=0)
            pltpu.make_async_copy(
                v_hbm.at[pl.ds(base + j * r, r)], vbuf.at[slot, pl.ds(j * r, r)],
                sems.at[1, slot]).start(priority=1)

    def wait(slot):
        pltpu.make_async_copy(kbuf.at[slot], kbuf.at[slot], sems.at[0, slot]).wait()
        pltpu.make_async_copy(vbuf.at[slot], vbuf.at[slot], sems.at[1, slot]).wait()

    for j in range(nslot - 1):
        start(j, j)

    ones = jnp.ones((M, 128), jnp.bfloat16)

    def body(i, carry):
        slot = i % nslot

        @pl.when(i + nslot - 1 < n)
        def _():
            start(i + nslot - 1, (i + nslot - 1) % nslot)

        sblk = i % bph

        @pl.when(sblk == 0)
        def _():
            acc[...] = jnp.zeros_like(acc)
            zacc[...] = jnp.zeros_like(zacc)

        wait(slot)
        om = om_ref[...]
        k = kbuf[slot]
        v = vbuf[slot]
        kp = jax.lax.dot_general(om, k, _NT, preferred_element_type=jnp.float32)
        kf = k.astype(jnp.float32)
        sq = kf * kf
        sqh = sq[:, 0:128]
        for j in range(1, D // 128):
            sqh = sqh + sq[:, j * 128:(j + 1) * 128]
        ksq = jax.lax.dot_general(ones, sqh.astype(jnp.bfloat16), _NT,
                                  preferred_element_type=jnp.float32)
        phi = jnp.exp(kp * scale - ksq * (0.5 * scale * scale)) * ism + 1e-6
        zz = phi[:, 0:128]
        for j in range(1, R // 128):
            zz = zz + phi[:, j * 128:(j + 1) * 128]
        zacc[...] += zz
        acc[...] += jax.lax.dot_general(phi.astype(jnp.bfloat16), v, _NN,
                                        preferred_element_type=jnp.float32)

        @pl.when(sblk == bph - 1)
        def _():
            h = i // bph
            qs = q_ref[h].astype(jnp.float32) * scale
            omf = om_ref[...].astype(jnp.float32)
            qp = jnp.sum(omf * qs, axis=1, keepdims=True)
            qsq = 0.5 * jnp.sum(qs * qs, axis=1, keepdims=True)
            phiq = jnp.exp(qp - qsq) * ism + 1e-6
            num = jnp.sum(phiq * acc[...], axis=0, keepdims=True)
            z = jnp.sum(zacc[...], axis=1, keepdims=True)
            den = jnp.sum(phiq * z, axis=0, keepdims=True) + 1e-6
            o_ref[h] = (num / den).astype(o_ref.dtype)

        return carry

    jax.lax.fori_loop(0, n, body, 0)


@jax.jit
def pallas_standalone__linear_kernel_rfa__decode_kernel(
    q: jax.Array,
    k: jax.Array,
    v: jax.Array,
    omega: jax.Array,
):
    B, H, Sk, D = k.shape
    Sq = q.shape[2]
    M = omega.shape[0]
    assert Sq == 1 and Sk % _R == 0 and _R % _SUB == 0 and D % 128 == 0
    assert (B * H * Sk) // _R >= _NSLOT
    k2 = k.reshape(B * H * Sk, D)
    v2 = v.reshape(B * H * Sk, D)
    q3 = q.reshape(B * H, 1, D)
    out = pl.pallas_call(
        functools.partial(_rfa_kernel, Sk=Sk),
        in_specs=[
            pl.BlockSpec(memory_space=pltpu.VMEM),
            pl.BlockSpec(memory_space=pltpu.VMEM),
            pl.BlockSpec(memory_space=pl.ANY),
            pl.BlockSpec(memory_space=pl.ANY),
        ],
        out_specs=pl.BlockSpec(memory_space=pltpu.VMEM),
        out_shape=jax.ShapeDtypeStruct((B * H, 1, D), q.dtype),
        scratch_shapes=[
            pltpu.VMEM((_NSLOT, _R, D), k.dtype),
            pltpu.VMEM((_NSLOT, _R, D), v.dtype),
            pltpu.SemaphoreType.DMA((2, _NSLOT)),
            pltpu.VMEM((M, D), jnp.float32),
            pltpu.VMEM((M, 128), jnp.float32),
        ],
        compiler_params=pltpu.CompilerParams(vmem_limit_bytes=64 * 1024 * 1024),
    )(q3, omega, k2, v2)
    return out.reshape(B, H, Sq, D)
```

```python
import functools

import jax
import jax.numpy as jnp
import jax.experimental.pallas as pl
import jax.experimental.pallas.tpu as pltpu

_NT = (((1,), (1,)), ((), ()))
_NN = (((1,), (0,)), ((), ()))

_R = 1024
_SUB = 64
_NSTREAM = 8
_NSLOT = 4


def _rfa_kernel(q_hbm, om_hbm, k_hbm, v_hbm, o_ref,
                kbuf, vbuf, sems, acc, zacc, qf, of, qv, omv, sio, *, Sk):
    D = k_hbm.shape[-1]
    M = om_hbm.shape[0]
    R, r, ns, nslot = _R, _SUB, _NSTREAM, _NSLOT
    rs = R // ns
    nt = rs // r
    seg = Sk // ns
    bph = Sk // R
    n = k_hbm.shape[0] // R
    scale = float(D) ** -0.25
    ism = float(M) ** -0.5

    def start(i, slot):
        base = (i // bph) * Sk + (i % bph) * rs
        for j in range(nt):
            for s in range(ns):
                off = pl.multiple_of(base + (s * seg + j * r), r)
                dst = (j * ns + s) * r
                pltpu.make_async_copy(
                    k_hbm.at[pl.ds(off, r)], kbuf.at[slot, pl.ds(dst, r)],
                    sems.at[0, slot]).start(priority=0)
                pltpu.make_async_copy(
                    v_hbm.at[pl.ds(off, r)], vbuf.at[slot, pl.ds(dst, r)],
                    sems.at[1, slot]).start(priority=1)

    def wait(slot):
        pltpu.make_async_copy(kbuf.at[slot], kbuf.at[slot], sems.at[0, slot]).wait()
        pltpu.make_async_copy(vbuf.at[slot], vbuf.at[slot], sems.at[1, slot]).wait()

    start(0, 0)
    cq = pltpu.make_async_copy(q_hbm, qv, sio.at[0])
    co = pltpu.make_async_copy(om_hbm, omv, sio.at[1])
    cq.start()
    co.start()
    for j in range(1, nslot - 1):
        start(j, j)
    cq.wait()
    co.wait()
    qf[...] = qv[...].astype(jnp.float32) * scale

    ones = jnp.ones((M, 128), jnp.bfloat16)

    def body(i, carry):
        slot = i % nslot

        @pl.when(i + nslot - 1 < n)
        def _():
            start(i + nslot - 1, (i + nslot - 1) % nslot)

        sblk = i % bph

        @pl.when(sblk == 0)
        def _():
            acc[...] = jnp.zeros_like(acc)
            zacc[...] = jnp.zeros_like(zacc)

        wait(slot)
        k = kbuf[slot]
        v = vbuf[slot]
        kp = jax.lax.dot_general(omv[...], k, _NT, preferred_element_type=jnp.float32)
        kf = k.astype(jnp.float32)
        sq = kf * kf
        sqh = sq[:, 0:128]
        for c in range(1, D // 128):
            sqh = sqh + sq[:, c * 128:(c + 1) * 128]
        ksq = jax.lax.dot_general(ones, sqh.astype(jnp.bfloat16), _NT,
                                  preferred_element_type=jnp.float32)
        phi = jnp.exp(kp * scale - ksq * (0.5 * scale * scale)) * ism + 1e-6
        phib = phi.astype(jnp.bfloat16)
        phif = phib.astype(jnp.float32)
        zz = phif[:, 0:128]
        for c in range(1, R // 128):
            zz = zz + phif[:, c * 128:(c + 1) * 128]
        zacc[...] += zz
        acc[...] += jax.lax.dot_general(phib, v, _NN, preferred_element_type=jnp.float32)

        @pl.when(sblk == bph - 1)
        def _():
            hh = i // bph
            qs = qf[pl.ds(hh, 1), :]
            omf = omv[...].astype(jnp.float32)
            qp = jnp.sum(omf * qs, axis=1, keepdims=True)
            qsq = 0.5 * jnp.sum(qs * qs, axis=1, keepdims=True)
            phiq = jnp.exp(qp - qsq) * ism + 1e-6
            num = jnp.sum(phiq * acc[...], axis=0, keepdims=True)
            z = jnp.sum(zacc[...], axis=1, keepdims=True)
            den = jnp.sum(phiq * z, axis=0, keepdims=True) + 1e-6
            of[pl.ds(hh, 1), :] = num / den

        return carry

    jax.lax.fori_loop(0, n, body, 0)
    o_ref[...] = of[...].astype(o_ref.dtype)


@jax.jit
def pallas_standalone__linear_kernel_rfa__decode_kernel(
    q: jax.Array,
    k: jax.Array,
    v: jax.Array,
    omega: jax.Array,
):
    B, H, Sk, D = k.shape
    Sq = q.shape[2]
    M = omega.shape[0]
    assert Sq == 1 and D % 128 == 0
    assert Sk % _R == 0 and _R % (_SUB * _NSTREAM) == 0
    assert (B * H * Sk) // _R >= _NSLOT
    k2 = k.reshape(B * H * Sk, D)
    v2 = v.reshape(B * H * Sk, D)
    q2 = q.reshape(B * H, D)
    out = pl.pallas_call(
        functools.partial(_rfa_kernel, Sk=Sk),
        in_specs=[pl.BlockSpec(memory_space=pl.ANY)] * 4,
        out_specs=pl.BlockSpec(memory_space=pltpu.VMEM),
        out_shape=jax.ShapeDtypeStruct((B * H, D), q.dtype),
        scratch_shapes=[
            pltpu.VMEM((_NSLOT, _R, D), k.dtype),
            pltpu.VMEM((_NSLOT, _R, D), v.dtype),
            pltpu.SemaphoreType.DMA((2, _NSLOT)),
            pltpu.VMEM((M, D), jnp.float32),
            pltpu.VMEM((M, 128), jnp.float32),
            pltpu.VMEM((B * H, D), jnp.float32),
            pltpu.VMEM((B * H, D), jnp.float32),
            pltpu.VMEM((B * H, D), q.dtype),
            pltpu.VMEM((M, D), omega.dtype),
            pltpu.SemaphoreType.DMA((2,)),
        ],
        compiler_params=pltpu.CompilerParams(vmem_limit_bytes=64 * 1024 * 1024),
    )(q2, omega, k2, v2)
    return out.reshape(B, H, Sq, D)
```

```python
import functools

import jax
import jax.numpy as jnp
import jax.experimental.pallas as pl
import jax.experimental.pallas.tpu as pltpu

_NT = (((1,), (1,)), ((), ()))
_NN = (((1,), (0,)), ((), ()))

_SPLITS = (32, 96)
_NSTREAM = 8
_PHASE = 80
_NSLOT = 4
_RS = sum(_SPLITS)
_R = _RS * _NSTREAM


def _rfa_kernel(q_hbm, om_hbm, k_hbm, v_hbm, o_ref,
                kbuf, vbuf, sems, acc, zacc, qf, of, qv, omv, sio, *, Sk):
    D = k_hbm.shape[-1]
    M = om_hbm.shape[0]
    R, rs, ns, nslot, p = _R, _RS, _NSTREAM, _NSLOT, _PHASE
    offs = [sum(_SPLITS[:i]) for i in range(len(_SPLITS))]
    seg = Sk // ns
    bph = Sk // R
    n = k_hbm.shape[0] // R
    scale = float(D) ** -0.25
    ism = float(M) ** -0.5

    def copy(src_row, dst_row, nrows, slot):
        if not isinstance(src_row, int):
            src_row = pl.multiple_of(src_row, 16)
        pltpu.make_async_copy(
            k_hbm.at[pl.ds(src_row, nrows)], kbuf.at[slot, pl.ds(dst_row, nrows)],
            sems.at[0, slot]).start(priority=0)
        pltpu.make_async_copy(
            v_hbm.at[pl.ds(src_row, nrows)], vbuf.at[slot, pl.ds(dst_row, nrows)],
            sems.at[1, slot]).start(priority=1)

    def when(cond, fn):
        if isinstance(cond, bool):
            if cond:
                fn()
        else:
            pl.when(cond)(fn)

    def start(i, slot):
        hbase = (i // bph) * Sk
        sb = i % bph
        base = hbase + sb * rs + p
        for o, r in zip(offs, _SPLITS):
            for s in range(ns):
                dst = s * rs + o
                if s == ns - 1 and p + o + r > rs:
                    def normal(o=o, r=r, dst=dst, s=s):
                        copy(base + (s * seg + o), dst, r, slot)

                    def wrapped(o=o, r=r, dst=dst, s=s):
                        n1 = max(rs - (p + o), 0)
                        if n1 > 0:
                            copy(base + (s * seg + o), dst, n1, slot)
                        copy(hbase + (p + o + n1 - rs), dst + n1, r - n1, slot)

                    when(sb != bph - 1, normal)
                    when(sb == bph - 1, wrapped)
                else:
                    copy(base + (s * seg + o), dst, r, slot)

    def wait(slot):
        pltpu.make_async_copy(kbuf.at[slot], kbuf.at[slot], sems.at[0, slot]).wait()
        pltpu.make_async_copy(vbuf.at[slot], vbuf.at[slot], sems.at[1, slot]).wait()

    start(0, 0)
    cq = pltpu.make_async_copy(q_hbm, qv, sio.at[0])
    co = pltpu.make_async_copy(om_hbm, omv, sio.at[1])
    cq.start()
    co.start()
    for j in range(1, nslot - 1):
        start(j, j)
    cq.wait()
    co.wait()
    qf[...] = qv[...].astype(jnp.float32) * scale

    ones = jnp.ones((M, 128), jnp.bfloat16)

    def body(i, carry):
        slot = i % nslot

        @pl.when(i + nslot - 1 < n)
        def _():
            start(i + nslot - 1, (i + nslot - 1) % nslot)

        sblk = i % bph

        @pl.when(sblk == 0)
        def _():
            acc[...] = jnp.zeros_like(acc)
            zacc[...] = jnp.zeros_like(zacc)

        wait(slot)
        k = kbuf[slot]
        v = vbuf[slot]
        kp = jax.lax.dot_general(omv[...], k, _NT, preferred_element_type=jnp.float32)
        kf = k.astype(jnp.float32)
        sq = kf * kf
        sqh = sq[:, 0:128]
        for c in range(1, D // 128):
            sqh = sqh + sq[:, c * 128:(c + 1) * 128]
        ksq = jax.lax.dot_general(ones, sqh.astype(jnp.bfloat16), _NT,
                                  preferred_element_type=jnp.float32)
        phi = jnp.exp(kp * scale - ksq * (0.5 * scale * scale)) * ism + 1e-6
        phib = phi.astype(jnp.bfloat16)
        phif = phib.astype(jnp.float32)
        zz = phif[:, 0:128]
        for c in range(1, R // 128):
            zz = zz + phif[:, c * 128:(c + 1) * 128]
        zacc[...] += zz
        acc[...] += jax.lax.dot_general(phib, v, _NN, preferred_element_type=jnp.float32)

        @pl.when(sblk == bph - 1)
        def _():
            hh = i // bph
            qs = qf[pl.ds(hh, 1), :]
            omf = omv[...].astype(jnp.float32)
            qp = jnp.sum(omf * qs, axis=1, keepdims=True)
            qsq = 0.5 * jnp.sum(qs * qs, axis=1, keepdims=True)
            phiq = jnp.exp(qp - qsq) * ism + 1e-6
            num = jnp.sum(phiq * acc[...], axis=0, keepdims=True)
            z = jnp.sum(zacc[...], axis=1, keepdims=True)
            den = jnp.sum(phiq * z, axis=0, keepdims=True) + 1e-6
            of[pl.ds(hh, 1), :] = num / den

        return carry

    jax.lax.fori_loop(0, n, body, 0)
    o_ref[...] = of[...].astype(o_ref.dtype)


@jax.jit
def pallas_standalone__linear_kernel_rfa__decode_kernel(
    q: jax.Array,
    k: jax.Array,
    v: jax.Array,
    omega: jax.Array,
):
    B, H, Sk, D = k.shape
    Sq = q.shape[2]
    M = omega.shape[0]
    assert Sq == 1 and D % 128 == 0 and Sk % _R == 0
    assert all(x % 16 == 0 for x in _SPLITS) and _PHASE % 16 == 0 and 0 <= _PHASE < _RS
    assert (B * H * Sk) // _R >= _NSLOT
    k2 = k.reshape(B * H * Sk, D)
    v2 = v.reshape(B * H * Sk, D)
    q2 = q.reshape(B * H, D)
    out = pl.pallas_call(
        functools.partial(_rfa_kernel, Sk=Sk),
        in_specs=[pl.BlockSpec(memory_space=pl.ANY)] * 4,
        out_specs=pl.BlockSpec(memory_space=pltpu.VMEM),
        out_shape=jax.ShapeDtypeStruct((B * H, D), q.dtype),
        scratch_shapes=[
            pltpu.VMEM((_NSLOT, _R, D), k.dtype),
            pltpu.VMEM((_NSLOT, _R, D), v.dtype),
            pltpu.SemaphoreType.DMA((2, _NSLOT)),
            pltpu.VMEM((M, D), jnp.float32),
            pltpu.VMEM((M, 128), jnp.float32),
            pltpu.VMEM((B * H, D), jnp.float32),
            pltpu.VMEM((B * H, D), jnp.float32),
            pltpu.VMEM((B * H, D), q.dtype),
            pltpu.VMEM((M, D), omega.dtype),
            pltpu.SemaphoreType.DMA((2,)),
        ],
        compiler_params=pltpu.CompilerParams(vmem_limit_bytes=64 * 1024 * 1024),
    )(q2, omega, k2, v2)
    return out.reshape(B, H, Sq, D)
```

```python
import functools

import jax
import jax.numpy as jnp
import jax.experimental.pallas as pl
import jax.experimental.pallas.tpu as pltpu

_NT = (((1,), (1,)), ((), ()))
_NN = (((1,), (0,)), ((), ()))

_SPLITS = (16, 16, 96)
_NSTREAM = 8
_PHASE = 64
_NSLOT = 4
_RS = sum(_SPLITS)
_R = _RS * _NSTREAM


def _rfa_kernel(q_hbm, om_hbm, k_hbm, v_hbm, o_ref,
                kbuf, vbuf, sems, acc, zacc, qf, of, qv, omv, sio, *, Sk):
    D = k_hbm.shape[-1]
    M = om_hbm.shape[0]
    R, rs, ns, nslot, p = _R, _RS, _NSTREAM, _NSLOT, _PHASE
    offs = [sum(_SPLITS[:i]) for i in range(len(_SPLITS))]
    seg = Sk // ns
    bph = Sk // R
    n = k_hbm.shape[0] // R
    scale = float(D) ** -0.25
    ism = float(M) ** -0.5

    def copy(src_row, dst_row, nrows, slot):
        if not isinstance(src_row, int):
            src_row = pl.multiple_of(src_row, 16)
        pltpu.make_async_copy(
            k_hbm.at[pl.ds(src_row, nrows)], kbuf.at[slot, pl.ds(dst_row, nrows)],
            sems.at[0, slot]).start(priority=0)
        pltpu.make_async_copy(
            v_hbm.at[pl.ds(src_row, nrows)], vbuf.at[slot, pl.ds(dst_row, nrows)],
            sems.at[1, slot]).start(priority=1)

    def when(cond, fn):
        if isinstance(cond, bool):
            if cond:
                fn()
        else:
            pl.when(cond)(fn)

    def start(i, slot):
        hbase = (i // bph) * Sk
        sb = i % bph
        base = hbase + sb * rs + p
        for o, r in zip(offs, _SPLITS):
            for s in range(ns):
                dst = s * rs + o
                if s == ns - 1 and p + o + r > rs:
                    def normal(o=o, r=r, dst=dst, s=s):
                        src = base + (s * seg + o)
                        if isinstance(src, int):
                            src = min(src, n * R - r)
                        else:
                            src = jnp.minimum(src, n * R - r)
                        copy(src, dst, r, slot)

                    def wrapped(o=o, r=r, dst=dst, s=s):
                        n1 = max(rs - (p + o), 0)
                        if n1 > 0:
                            copy(base + (s * seg + o), dst, n1, slot)
                        copy(hbase + (p + o + n1 - rs), dst + n1, r - n1, slot)

                    when(sb != bph - 1, normal)
                    when(sb == bph - 1, wrapped)
                else:
                    copy(base + (s * seg + o), dst, r, slot)

    def wait(slot):
        pltpu.make_async_copy(kbuf.at[slot], kbuf.at[slot], sems.at[0, slot]).wait()
        pltpu.make_async_copy(vbuf.at[slot], vbuf.at[slot], sems.at[1, slot]).wait()

    start(0, 0)
    cq = pltpu.make_async_copy(q_hbm, qv, sio.at[0])
    co = pltpu.make_async_copy(om_hbm, omv, sio.at[1])
    cq.start()
    co.start()
    for j in range(1, nslot - 1):
        start(j, j)
    cq.wait()
    co.wait()
    qf[...] = qv[...].astype(jnp.float32) * scale

    ones = jnp.ones((M, 128), jnp.bfloat16)

    def body(i, carry):
        slot = i % nslot

        @pl.when(i + nslot - 1 < n)
        def _():
            start(i + nslot - 1, (i + nslot - 1) % nslot)

        sblk = i % bph

        @pl.when(sblk == 0)
        def _():
            acc[...] = jnp.zeros_like(acc)
            zacc[...] = jnp.zeros_like(zacc)

        wait(slot)
        k = kbuf[slot]
        v = vbuf[slot]
        kp = jax.lax.dot_general(omv[...], k, _NT, preferred_element_type=jnp.float32)
        kf = k.astype(jnp.float32)
        sq = kf * kf
        sqh = sq[:, 0:128]
        for c in range(1, D // 128):
            sqh = sqh + sq[:, c * 128:(c + 1) * 128]
        ksq = jax.lax.dot_general(ones, sqh.astype(jnp.bfloat16), _NT,
                                  preferred_element_type=jnp.float32)
        phi = jnp.exp(kp * scale - ksq * (0.5 * scale * scale)) * ism + 1e-6
        phib = phi.astype(jnp.bfloat16)
        phif = phib.astype(jnp.float32)
        zz = phif[:, 0:128]
        for c in range(1, R // 128):
            zz = zz + phif[:, c * 128:(c + 1) * 128]
        zacc[...] += zz
        acc[...] += jax.lax.dot_general(phib, v, _NN, preferred_element_type=jnp.float32)

        @pl.when(sblk == bph - 1)
        def _():
            hh = i // bph
            qs = qf[pl.ds(hh, 1), :]
            omf = omv[...].astype(jnp.float32)
            qp = jnp.sum(omf * qs, axis=1, keepdims=True)
            qsq = 0.5 * jnp.sum(qs * qs, axis=1, keepdims=True)
            phiq = jnp.exp(qp - qsq) * ism + 1e-6
            num = jnp.sum(phiq * acc[...], axis=0, keepdims=True)
            z = jnp.sum(zacc[...], axis=1, keepdims=True)
            den = jnp.sum(phiq * z, axis=0, keepdims=True) + 1e-6
            of[pl.ds(hh, 1), :] = num / den

        return carry

    jax.lax.fori_loop(0, n, body, 0)
    o_ref[...] = of[...].astype(o_ref.dtype)


@jax.jit
def pallas_standalone__linear_kernel_rfa__decode_kernel(
    q: jax.Array,
    k: jax.Array,
    v: jax.Array,
    omega: jax.Array,
):
    B, H, Sk, D = k.shape
    Sq = q.shape[2]
    M = omega.shape[0]
    assert Sq == 1 and D % 128 == 0 and Sk % _R == 0
    assert all(x % 16 == 0 for x in _SPLITS) and _PHASE % 16 == 0 and 0 <= _PHASE < _RS
    assert (B * H * Sk) // _R >= _NSLOT
    k2 = k.reshape(B * H * Sk, D)
    v2 = v.reshape(B * H * Sk, D)
    q2 = q.reshape(B * H, D)
    out = pl.pallas_call(
        functools.partial(_rfa_kernel, Sk=Sk),
        in_specs=[pl.BlockSpec(memory_space=pl.ANY)] * 4,
        out_specs=pl.BlockSpec(memory_space=pltpu.VMEM),
        out_shape=jax.ShapeDtypeStruct((B * H, D), q.dtype),
        scratch_shapes=[
            pltpu.VMEM((_NSLOT, _R, D), k.dtype),
            pltpu.VMEM((_NSLOT, _R, D), v.dtype),
            pltpu.SemaphoreType.DMA((2, _NSLOT)),
            pltpu.VMEM((M, D), jnp.float32),
            pltpu.VMEM((M, 128), jnp.float32),
            pltpu.VMEM((B * H, D), jnp.float32),
            pltpu.VMEM((B * H, D), jnp.float32),
            pltpu.VMEM((B * H, D), q.dtype),
            pltpu.VMEM((M, D), omega.dtype),
            pltpu.SemaphoreType.DMA((2,)),
        ],
        compiler_params=pltpu.CompilerParams(vmem_limit_bytes=64 * 1024 * 1024),
    )(q2, omega, k2, v2)
    return out.reshape(B, H, Sq, D)
```

```python
import functools

import jax
import jax.numpy as jnp
import jax.experimental.pallas as pl
import jax.experimental.pallas.tpu as pltpu

_NT = (((1,), (1,)), ((), ()))
_NN = (((1,), (0,)), ((), ()))

_SPLITS = (16, 16, 96)
_NSTREAM = 8
_PHASE = 64
_NSLOT = 4
_RS = sum(_SPLITS)
_R = _RS * _NSTREAM


def _rfa_kernel(q_hbm, om_hbm, k_hbm, v_hbm, o_ref,
                kbuf, vbuf, sems, acc, zacc, qf, of, qv, omv, sio, *, Sk):
    D = k_hbm.shape[-1]
    M = om_hbm.shape[0]
    R, rs, ns, nslot, p = _R, _RS, _NSTREAM, _NSLOT, _PHASE
    offs = [sum(_SPLITS[:i]) for i in range(len(_SPLITS))]
    seg = Sk // ns
    bph = Sk // R
    n = k_hbm.shape[0] // R
    scale = float(D) ** -0.25
    ism = float(M) ** -0.5

    def copy(src_row, dst_row, nrows, slot):
        if not isinstance(src_row, int):
            src_row = pl.multiple_of(src_row, 16)
        pltpu.make_async_copy(
            k_hbm.at[pl.ds(src_row, nrows)], kbuf.at[slot, pl.ds(dst_row, nrows)],
            sems.at[0, slot]).start(priority=0)
        pltpu.make_async_copy(
            v_hbm.at[pl.ds(src_row, nrows)], vbuf.at[slot, pl.ds(dst_row, nrows)],
            sems.at[1, slot]).start(priority=1)

    def when(cond, fn):
        if isinstance(cond, bool):
            if cond:
                fn()
        else:
            pl.when(cond)(fn)

    def start(i, slot):
        hbase = (i // bph) * Sk
        sb = i % bph
        base = hbase + sb * rs + p
        for o, r in zip(offs, _SPLITS):
            for s in range(ns):
                dst = s * rs + o
                if s == ns - 1 and p + o + r > rs:
                    def normal(o=o, r=r, dst=dst, s=s):
                        src = base + (s * seg + o)
                        if isinstance(src, int):
                            src = min(src, n * R - r)
                        else:
                            src = jnp.minimum(src, n * R - r)
                        copy(src, dst, r, slot)

                    def wrapped(o=o, r=r, dst=dst, s=s):
                        n1 = max(rs - (p + o), 0)
                        if n1 > 0:
                            copy(base + (s * seg + o), dst, n1, slot)
                        copy(hbase + (p + o + n1 - rs), dst + n1, r - n1, slot)

                    when(sb != bph - 1, normal)
                    when(sb == bph - 1, wrapped)
                else:
                    copy(base + (s * seg + o), dst, r, slot)

    def wait(slot):
        pltpu.make_async_copy(kbuf.at[slot], kbuf.at[slot], sems.at[0, slot]).wait()
        pltpu.make_async_copy(vbuf.at[slot], vbuf.at[slot], sems.at[1, slot]).wait()

    start(0, 0)
    cq = pltpu.make_async_copy(q_hbm, qv, sio.at[0])
    co = pltpu.make_async_copy(om_hbm, omv, sio.at[1])
    cq.start()
    co.start()
    for j in range(1, nslot - 1):
        start(j, j)
    cq.wait()
    co.wait()
    qf[...] = qv[...].astype(jnp.float32) * scale

    ones = jnp.ones((M, 128), jnp.bfloat16)

    def body(i, carry):
        slot = i % nslot

        @pl.when(i + nslot - 1 < n)
        def _():
            start(i + nslot - 1, (i + nslot - 1) % nslot)

        sblk = i % bph

        @pl.when(sblk == 0)
        def _():
            acc[...] = jnp.zeros_like(acc)
            zacc[...] = jnp.zeros_like(zacc)

        wait(slot)
        k = kbuf[slot]
        v = vbuf[slot]
        kp = jax.lax.dot_general(omv[...], k, _NT, preferred_element_type=jnp.float32)
        kf = k.astype(jnp.float32)
        sq = kf * kf
        sqh = sq[:, 0:128]
        for c in range(1, D // 128):
            sqh = sqh + sq[:, c * 128:(c + 1) * 128]
        ksq = jax.lax.dot_general(ones, sqh.astype(jnp.bfloat16), _NT,
                                  preferred_element_type=jnp.float32)
        phi = jnp.exp(kp * scale - ksq * (0.5 * scale * scale)) * ism + 1e-6
        phib = phi.astype(jnp.bfloat16)
        phif = phib.astype(jnp.float32)
        zz = phif[:, 0:128]
        for c in range(1, R // 128):
            zz = zz + phif[:, c * 128:(c + 1) * 128]
        zacc[...] += zz
        acc[...] += jax.lax.dot_general(phib, v, _NN, preferred_element_type=jnp.float32)

        @pl.when(sblk == bph - 1)
        def _():
            hh = i // bph
            qs = qf[pl.ds(hh, 1), :]
            omf = omv[...].astype(jnp.float32)
            qp = jnp.sum(omf * qs, axis=1, keepdims=True)
            qsq = 0.5 * jnp.sum(qs * qs, axis=1, keepdims=True)
            phiq = jnp.exp(qp - qsq) * ism + 1e-6
            num = jnp.sum(phiq * acc[...], axis=0, keepdims=True)
            z = jnp.sum(zacc[...], axis=1, keepdims=True)
            den = jnp.sum(phiq * z, axis=0, keepdims=True) + 1e-6
            of[pl.ds(hh, 1), :] = num / den

        return carry

    jax.lax.fori_loop(0, n, body, 0)
    o_ref[...] = of[...].astype(o_ref.dtype)


@jax.jit
def pallas_standalone__linear_kernel_rfa__decode_kernel(
    q: jax.Array,
    k: jax.Array,
    v: jax.Array,
    omega: jax.Array,
):
    B, H, Sk, D = k.shape
    Sq = q.shape[2]
    M = omega.shape[0]
    assert Sq == 1 and D % 128 == 0 and Sk % _R == 0
    assert all(x % 16 == 0 for x in _SPLITS) and _PHASE % 16 == 0 and 0 <= _PHASE < _RS
    assert (B * H * Sk) // _R >= _NSLOT
    k2 = k.reshape(B * H * Sk, D)
    v2 = v.reshape(B * H * Sk, D)
    q2 = q.reshape(B * H, D)
    out = pl.pallas_call(
        functools.partial(_rfa_kernel, Sk=Sk),
        in_specs=[pl.BlockSpec(memory_space=pl.ANY)] * 4,
        out_specs=pl.BlockSpec(memory_space=pltpu.VMEM),
        out_shape=jax.ShapeDtypeStruct((B * H, D), q.dtype),
        scratch_shapes=[
            pltpu.VMEM((_NSLOT, _R, D), k.dtype),
            pltpu.VMEM((_NSLOT, _R, D), v.dtype),
            pltpu.SemaphoreType.DMA((2, _NSLOT)),
            pltpu.VMEM((M, D), jnp.float32),
            pltpu.VMEM((M, 128), jnp.float32),
            pltpu.VMEM((B * H, D), jnp.float32),
            pltpu.VMEM((B * H, D), jnp.float32),
            pltpu.VMEM((B * H, D), q.dtype),
            pltpu.VMEM((M, D), omega.dtype),
            pltpu.SemaphoreType.DMA((2,)),
        ],
        compiler_params=pltpu.CompilerParams(
            vmem_limit_bytes=64 * 1024 * 1024,
            disable_bounds_checks=True,
        ),
    )(q2, omega, k2, v2)
    return out.reshape(B, H, Sq, D)
```
